```python
import os as _os
_os.environ.setdefault("JAX_PLATFORMS", "cpu")
import jax
import jax.numpy as jnp

def _softmax(x, axis=-1):
    return jax.nn.softmax(x, axis=axis)
def _gelu(x):
    return jax.nn.gelu(x, approximate=True)
def _silu(x):
    return jax.nn.silu(x)
def _sigmoid(x):
    return jax.nn.sigmoid(x)
def _layernorm(x, axis=-1, eps=1e-5):
    m = jnp.mean(x, axis=axis, keepdims=True)
    v = jnp.var(x, axis=axis, keepdims=True)
    return (x - m) / jnp.sqrt(v + eps)
def _scatter_add(tgt, idx, src, axis=0):
    return tgt.at[idx].add(src)
def _segment_sum(src, seg, n):
    return jax.ops.segment_sum(src, seg, n)
class _Rng:
    def __init__(self, key):
        self._k = key
    def _next(self):
        self._k, sub = jax.random.split(self._k)
        return sub
    def normal(self, shape):
        return jax.random.normal(self._next(), shape, dtype=jnp.bfloat16)
    def randint(self, lo, hi, shape):
        return jax.random.randint(self._next(), shape, lo, hi, dtype=jnp.int32)
    def uniform(self, shape, lo=0.0, hi=1.0):
        return jax.random.uniform(self._next(), shape, jnp.bfloat16, lo, hi)
    def permutation(self, n):
        return jax.random.permutation(self._next(), n)


kernel_name = 'interleave_layers__grouped_kv_mqa__sliding_block__prompt'

def setup_inputs():
    _rng = _Rng(jax.random.key(int.from_bytes(__import__("os").urandom(4), "little")))
    _w = (lambda a: (lambda t: t.astype(jnp.bfloat16) if jnp.issubdtype(t.dtype, jnp.floating) else t)(jnp.asarray(a)))
    def _A_setup():
        B, S, D, H = 1, 2048, 448, 16
        Dh = D // H
        return {
            "x": _w((lambda *s: _rng.normal(s) * 0.05)(B, S, D)),
            "wq": _w((lambda *s: _rng.normal(s) * 0.05)(D, H * Dh)),
            "wk": _w((lambda *s: _rng.normal(s) * 0.05)(D, Dh)),
            "wv": _w((lambda *s: _rng.normal(s) * 0.05)(D, Dh)),
            "wo": _w((lambda *s: _rng.normal(s) * 0.05)(H * Dh, D)),
        }
    _A_in = _A_setup()

    def _B_setup():
        B, S, D = 1, 2048, 448
        return {
            "x": _w((lambda *s: _rng.normal(s) * 0.05)(B, S, D)),
            "wqkv": _w((lambda *s: _rng.normal(s) * 0.05)(D, 3 * D)),
            "wo": _w((lambda *s: _rng.normal(s) * 0.05)(D, D)),
        }
    _B_in = _B_setup()

    return {
        "A_x": _A_in["x"],
        "A_wq": _A_in["wq"],
        "A_wk": _A_in["wk"],
        "A_wv": _A_in["wv"],
        "A_wo": _A_in["wo"],
        "B_x": _B_in["x"],
        "B_wqkv": _B_in["wqkv"],
        "B_wo": _B_in["wo"],
    }

def reference(A_x, A_wq, A_wk, A_wv, A_wo, B_x, B_wqkv, B_wo):
    def _A_ref(x, wq, wk, wv, wo):
        B, S, D = x.shape
        H = 16
        Dh = D // H
        q = (lambda x, *d: x.transpose(*d))((x @ wq).reshape(B, S, H, Dh), 0, 2, 1, 3)
        k = x @ wk
        v = x @ wv
        scores = jnp.einsum("bhqd,bkd->bhqk", q, k) * (Dh ** -0.5)
        p = _softmax(scores, axis=-1)
        o = jnp.einsum("bhqk,bkd->bhqd", p, v)
        return (lambda x, *d: x.transpose(*d))(o, 0, 2, 1, 3).reshape(B, S, H * Dh) @ wo

    def _B_ref(x, wqkv, wo):
        B, S, D = x.shape
        H = 16; Dh = D // H; W = 256
        qkv = (lambda x, *d: x.transpose(*d))((x @ wqkv).reshape(B, S, 3, H, Dh), 2, 0, 3, 1, 4)
        q, k, v = qkv[0], qkv[1], qkv[2]
        scores = jnp.einsum("bhqd,bhkd->bhqk", q, k) * (Dh ** -0.5)
        idx = jnp.arange(S)
        mask = (idx[:, None] - idx[None, :] >= 0) & (idx[:, None] - idx[None, :] < W)
        scores = jnp.where(mask[None, None], scores, -1e9)
        p = _softmax(scores, axis=-1)
        o = jnp.einsum("bhqk,bhkd->bhqd", p, v)
        return (lambda x, *d: x.transpose(*d))(o, 0, 2, 1, 3).reshape(B, S, D) @ wo

    x = A_x
    x = x + _A_ref(_layernorm(x, axis=-1), A_wq, A_wk, A_wv, A_wo)
    x = x + _B_ref(_layernorm(x, axis=-1), B_wqkv, B_wo)
    x = x + _A_ref(_layernorm(x, axis=-1), A_wq, A_wk, A_wv, A_wo)
    x = x + _B_ref(_layernorm(x, axis=-1), B_wqkv, B_wo)
    return x
```

```python
import functools
import math

import jax
import jax.numpy as jnp
from jax import lax
import jax.experimental.pallas as pl
import jax.experimental.pallas.tpu as pltpu

H = 16
W = 256
HP = 32
T = 128
EPS = 1e-5
MASKED = -1e9
LOG2E = math.log2(math.e)
F32 = jnp.float32
BF16 = jnp.bfloat16


def _dot(a, b):
    return jnp.dot(a, b, preferred_element_type=F32)


def _layernorm_t(x):
    n = x.shape[0]
    mean = jnp.sum(x, axis=0, keepdims=True) * (1.0 / n)
    xc = x - mean
    var = jnp.sum(xc * xc, axis=0, keepdims=True) * (1.0 / n)
    return xc * lax.rsqrt(var + EPS)


def _pad_heads(dst_ref, dst0, src, nheads, dh):
    for h in range(nheads):
        dst_ref[dst0 + h * HP : dst0 + h * HP + dh, :] = src[h * dh : (h + 1) * dh, :]


def _kernel(
    xt_ref, wq_ref, wkt_ref, wvt_ref, woa_ref, wqkv_ref, wob_ref, out_ref,
    x_ref, tmp_ref, wa_ref, wb_ref, woat_ref, wobt_ref,
    q_ref, k_ref, v_ref, o_ref,
    *, S, D,
):
    dh = D // H
    scale = dh**-0.5 * LOG2E
    P = H * HP
    CH = 512

    tmp_ref[...] = jnp.zeros(tmp_ref.shape, F32)
    _pad_heads(tmp_ref, 0, wq_ref[...].astype(F32).T, H, dh)
    tmp_ref[P : P + dh, :] = wkt_ref[...].astype(F32)
    tmp_ref[P + HP : P + HP + dh, :] = wvt_ref[...].astype(F32)
    wa_ref[...] = tmp_ref[0 : P + 2 * HP, :].astype(BF16)

    tmp_ref[...] = jnp.zeros(tmp_ref.shape, F32)
    _pad_heads(tmp_ref, 0, wqkv_ref[...].astype(F32).T, 3 * H, dh)
    wb_ref[...] = tmp_ref[...].astype(BF16)

    for src_ref, dst_ref in ((woa_ref, woat_ref), (wob_ref, wobt_ref)):
        tmp_ref[0:P, :] = jnp.zeros((P, D), F32)
        _pad_heads(tmp_ref, 0, src_ref[...].astype(F32), H, dh)
        dst_ref[...] = tmp_ref[0:P, :].T.astype(BF16)

    x_ref[...] = xt_ref[...].astype(F32)

    def ones_row(v):
        row = lax.broadcasted_iota(jnp.int32, v.shape, 0)
        return jnp.where(row % HP == dh, 1.0, v)

    def project_a(c, _):
        cols = pl.ds(pl.multiple_of(c * CH, CH), CH)
        ln = _layernorm_t(x_ref[:, cols]).astype(BF16)
        y = _dot(wa_ref[...], ln)
        q_ref[:, cols] = (y[0:P] * scale).astype(BF16)
        k_ref[0, cols, 0:HP] = y[P : P + HP].T.astype(BF16)
        v_ref[0:HP, cols] = ones_row(y[P + HP : P + 2 * HP]).astype(BF16)

    def project_b(c, _):
        cols = pl.ds(pl.multiple_of(c * CH, CH), CH)
        ln = _layernorm_t(x_ref[:, cols]).astype(BF16)
        q_ref[:, cols] = (_dot(wb_ref[0:P, :], ln) * scale).astype(BF16)
        kt = _dot(wb_ref[P : 2 * P, :], ln)
        for g in range(P // T):
            k_ref[g, cols, :] = kt[g * T : (g + 1) * T].T.astype(BF16)
        v_ref[:, cols] = ones_row(_dot(wb_ref[2 * P : 3 * P, :], ln)).astype(BF16)

    def attend_a(i, _):
        BQ = 1024
        h, qb = i // (S // BQ), i % (S // BQ)
        rows = pl.ds(pl.multiple_of(h * HP, HP), HP)
        cols = pl.ds(pl.multiple_of(qb * BQ, BQ), BQ)
        s = _dot(k_ref[0, :, 0:HP], q_ref[rows, cols])
        m = jnp.max(s, axis=0, keepdims=True)
        p = jnp.exp2(s - m).astype(BF16)
        acc = _dot(v_ref[0:HP, :], p)
        o_ref[rows, cols] = (acc / acc[dh : dh + 1]).astype(BF16)

    def attend_b(g, _):
        G = T // HP
        key = lax.broadcasted_iota(jnp.int32, (T, G * T), 0)
        qry = lax.broadcasted_iota(jnp.int32, (T, G * T), 1) % T
        causal = key <= qry
        rows = pl.ds(pl.multiple_of(g * T, T), T)
        zero = jnp.zeros((HP, T), BF16)
        for qb in range(S // T):
            k0 = max(0, qb * T - W)
            k1 = (qb + 1) * T
            qt = q_ref[rows, qb * T : k1]
            qd = jnp.concatenate(
                [
                    jnp.concatenate(
                        [qt[j * HP : (j + 1) * HP] if i == j else zero for i in range(G)],
                        axis=0,
                    )
                    for j in range(G)
                ],
                axis=1,
            )
            s = _dot(k_ref[g, k0:k1, :], qd)
            last = s[k1 - k0 - T :]
            if k1 - k0 == W + T:
                edge = jnp.where(causal, last, s[0:T])
                mid = s[T:W]
            else:
                edge = jnp.where(causal, last, MASKED * LOG2E)
                mid = s[0 : k1 - k0 - T] if k1 - k0 > T else None
            m = jnp.max(edge, axis=0, keepdims=True)
            if mid is not None:
                m = jnp.maximum(m, jnp.max(mid, axis=0, keepdims=True))
            pe = jnp.exp2(edge - m)
            parts = []
            if k1 - k0 == W + T:
                parts.append(jnp.where(causal, 0.0, pe).astype(BF16))
            if mid is not None:
                parts.append(jnp.exp2(mid - m).astype(BF16))
            parts.append(jnp.where(causal, pe, 0.0).astype(BF16))
            p = jnp.concatenate(parts, axis=0)
            for j in range(G):
                hr = pl.ds(pl.multiple_of(g * T + j * HP, HP), HP)
                acc = _dot(v_ref[hr, k0:k1], p[:, j * T : (j + 1) * T])
                o_ref[hr, qb * T : k1] = (acc / acc[dh : dh + 1]).astype(BF16)

    def add_output(wot_ref):
        def body(c, _):
            cols = pl.ds(pl.multiple_of(c * CH, CH), CH)
            x_ref[:, cols] += _dot(wot_ref[...], o_ref[:, cols])

        lax.fori_loop(0, S // CH, body, None)

    def layer_pair(_, carry):
        lax.fori_loop(0, S // CH, project_a, None)
        lax.fori_loop(0, H * (S // 1024), attend_a, None)
        add_output(woat_ref)
        lax.fori_loop(0, S // CH, project_b, None)
        lax.fori_loop(0, P // T, attend_b, None)
        add_output(wobt_ref)

    lax.fori_loop(0, 2, layer_pair, None)
    out_ref[...] = x_ref[...].astype(out_ref.dtype)


@jax.jit
def pallas_interleave_layers__grouped_kv_mqa__sliding_block__prompt_kernel(
    A_x: jax.Array,
    A_wq: jax.Array,
    A_wk: jax.Array,
    A_wv: jax.Array,
    A_wo: jax.Array,
    B_x: jax.Array,
    B_wqkv: jax.Array,
    B_wo: jax.Array,
):
    del B_x
    _, S, D = A_x.shape
    P = H * HP
    out_t = pl.pallas_call(
        functools.partial(_kernel, S=S, D=D),
        out_shape=jax.ShapeDtypeStruct((D, S), A_x.dtype),
        scratch_shapes=[
            pltpu.VMEM((D, S), F32),
            pltpu.VMEM((3 * P, D), F32),
            pltpu.VMEM((P + 2 * HP, D), BF16),
            pltpu.VMEM((3 * P, D), BF16),
            pltpu.VMEM((D, P), BF16),
            pltpu.VMEM((D, P), BF16),
            pltpu.VMEM((P, S), BF16),
            pltpu.VMEM((P // T, S, T), BF16),
            pltpu.VMEM((P, S), BF16),
            pltpu.VMEM((P, S), BF16),
        ],
        compiler_params=pltpu.CompilerParams(vmem_limit_bytes=100 * 1024 * 1024),
    )(A_x[0].T, A_wq, A_wk.T, A_wv.T, A_wo, B_wqkv, B_wo)
    return out_t.T[None]
```

```python
import functools
import math

import jax
import jax.numpy as jnp
from jax import lax
import jax.experimental.pallas as pl
import jax.experimental.pallas.tpu as pltpu

H = 16
DH = 28
W = 256
EPS = 1e-5
LOG2E = math.log2(math.e)
QSCALE = DH**-0.5 * LOG2E
MASKED = -1e9 * LOG2E

T = 128
G = 4
GD = G * DH
NG = H // G
CH = 512
TC = CH // T
VK = 16
NV = 11
PART = 2
QW = T // G
LAG = T - QW
NB = W // QW + 1
FIRST = 6

F32 = jnp.float32
BF16 = jnp.bfloat16
U32 = jnp.uint32


def _dot(a, b):
    return jnp.dot(a, b, preferred_element_type=F32)


def _pack(x):
    return pltpu.bitcast(x.astype(BF16), U32)


def _pack_transposed(x):
    return pltpu.bitcast(x.astype(BF16).T, U32)


def _unpack(x):
    return pltpu.bitcast(x, BF16)


def _iota(shape, dim):
    return lax.broadcasted_iota(jnp.int32, shape, dim)


def _tile(t):
    return slice(t * T, (t + 1) * T)


def _layernorm(x):
    n = x.shape[0]
    xc = x - jnp.sum(x, axis=0, keepdims=True) * (1.0 / n)
    var = jnp.sum(xc * xc, axis=0, keepdims=True) * (1.0 / n)
    return xc * lax.rsqrt(var + EPS)


def _window(y, j):
    r0 = j * DH - 4 * (j % 2)
    return y[r0 : r0 + 32]


def _merge_pair(even, odd):
    mid = jnp.where(_iota((8, even.shape[1]), 0) < 4, even[24:32], odd[0:8])
    return jnp.concatenate([even[0:24], mid, odd[8:32]], axis=0)


def _with_ones(v, odd):
    return jnp.where(_iota(v.shape, 0) == (0 if odd else DH), 1.0, v)


def _normalize(acc, odd):
    row = 0 if odd else DH
    total = acc[row : row + 1]
    r = pltpu.reciprocal(total, approx=True)
    return acc * (r * (2.0 - total * r))


def _pad_rows(y):
    return jnp.concatenate([y, jnp.zeros((T - y.shape[0], y.shape[1]), y.dtype)], axis=0)


def _chain(*tasks):
    def gen():
        for _, task in tasks:
            yield from task

    return sum(cost for cost, _ in tasks), gen()


def _mixed(*tasks):
    def gen():
        live = [[0.0, cost, task] for cost, task in tasks]
        while live:
            behind = min(live, key=lambda entry: entry[0] / entry[1])
            piece = next(behind[2], None)
            if piece is None:
                live.remove(behind)
            else:
                behind[0] += piece
                yield piece

    return sum(cost for cost, _ in tasks), gen()


def _head(task, cost):
    def gen():
        done = 0
        while done < cost:
            piece = next(task[1])
            done += piece
            yield piece

    return cost, gen()


def _kernel(
    xt_hbm, wq_hbm, wkt_hbm, wvt_hbm, woa_hbm, wqkv_hbm, wob_hbm, out_hbm,
    xin_ref, wq_ref, wkt_ref, wvt_ref, woa_ref, wqkv_ref, wob_ref, out_ref,
    x_ref, wa_ref, wb_ref, woat_ref, wobt_ref,
    ka_ref, kv_ref, va_ref, qa_ref, qf0_ref, qf1_ref, qh0_ref, qh1_ref,
    q_ref, kb_ref, tail_ref, vb_ref, o_ref,
    s0_ref, s1_ref, m0_ref, m1_ref, fence_ref, in_sem, out_sem,
):
    D, S = x_ref.shape
    NT, NC = S // T, S // CH
    SPLIT = 8
    bufs = ((s0_ref, m0_ref), (s1_ref, m1_ref))
    qf_refs, qh_refs = (qf0_ref, qf1_ref), (qh0_ref, qh1_ref)
    vtiles = sorted(((n + 1) * NT // NV - 3) % NT for n in range(NV))

    def chunk(c):
        return pl.ds(c * CH if isinstance(c, int) else pl.multiple_of(c * CH, CH), CH)

    x_in = [
        pltpu.make_async_copy(xt_hbm.at[:, c], xin_ref.at[:, c], in_sem.at[i])
        for i, c in enumerate((slice(0, FIRST * T), slice(FIRST * T, S)))
    ]
    w_in = [
        pltpu.make_async_copy(src, dst, in_sem.at[2 + i])
        for i, (src, dst) in enumerate((
            (wq_hbm, wq_ref), (wkt_hbm, wkt_ref), (wvt_hbm, wvt_ref),
            (woa_hbm, woa_ref), (wqkv_hbm, wqkv_ref), (wob_hbm, wob_ref),
        ))
    ]
    x_out = [
        pltpu.make_async_copy(out_ref.at[:, chunk(c)], out_hbm.at[:, chunk(c)], out_sem.at[c])
        for c in range(NC)
    ]

    d1, d2 = D - T, D - T // 2
    depth = ((0, d2), (d2 - T, d1), (d2, D), (d1, D))

    def stage_weights(src_ref, dst_ref):
        n = src_ref.shape[1]
        for c0 in range(0, n, T):
            c1 = min(c0 + T, n)
            w = jnp.concatenate([src_ref[a:b, c0:c1] for a, b in depth], axis=0)
            dst_ref[c0 // 2 : c1 // 2, :] = _pack_transposed(w)
            yield 1

    def split(one, two):
        shared = jnp.concatenate([two[d1:d2], one[d2:]], axis=0).astype(BF16)
        back = shared.astype(F32)
        one = jnp.concatenate([one[:d1], one[d1:d2] - back[: d2 - d1]], axis=0)
        two = jnp.concatenate([two[:d1], two[d2:] - back[d2 - d1 :]], axis=0)
        return one.astype(BF16), two.astype(BF16), shared

    def multiply(w_ref, rows, x):
        one, two, shared = x
        w_two = jnp.concatenate([w_ref[rows, : d2 - T], w_ref[rows, d2 : d2 + T]], axis=1)
        first = _dot(_unpack(w_ref[rows, :d2]), one)
        both = _dot(_unpack(w_ref[rows, d2 + T :]), shared)
        return first + both, _dot(_unpack(w_two), two) + both

    def each_group(w_ref, g0, t, x, consume, at_once=1):
        for g in range(0, NG, at_once):
            rows = slice((g0 + g) * GD // 2, (g0 + g + at_once) * GD // 2)
            for i, y in enumerate(multiply(w_ref, rows, x)):
                for e in range(at_once):
                    consume(g + e, t + i, y[e * GD : (e + 1) * GD])
                    yield GD

    def tile_pairs(task, prepare, t0, t1):
        operands = prepare(t0)
        for t in range(t0, t1, 2):
            pieces = task(t, operands)
            yield next(pieces)
            if t + 2 < t1:
                operands = prepare(t + 2)
            yield from pieces

    def normed(t):
        return split(*(_layernorm(x_ref[:, _tile(t + i)]) for i in range(2)))

    def attended(t):
        def one(t):
            heads = [_normalize(o_ref[h, :, _tile(t)], h % 2) for h in range(H)]
            return jnp.concatenate(
                [_merge_pair(heads[h], heads[h + 1]) for h in range(0, H, 2)], axis=0
            )

        return split(one(t), one(t + 1))

    def stage_queries(par, u, q):
        qf_refs[par][:, _tile(u)] = _unpack(q).astype(F32)
        for j in range(G):
            rolled = pltpu.roll(q, (G - j) * DH // 2, 0) if j else q
            qh_refs[par][j, :, _tile(u)] = rolled[0:16]

    def project_a(t0, ln):
        for t, y in enumerate(multiply(wa_ref, slice(D // 2, D // 2 + 32), ln), t0):
            ka_ref[t * T // 2 : (t + 1) * T // 2, :] = _pack_transposed(_pad_rows(y[0:32]))
            if t in vtiles:
                mine = _iota((8, T), 1) // VK == _iota((8, T), 0)
                for d in range(0, DH, 8):
                    row = pltpu.roll(y[d : d + 8], VK, 1, stride=VK, stride_axis=0)
                    row = jnp.sum(jnp.where(mine, row, 0.0), axis=0, keepdims=True)
                    n = min(8, DH - d) * VK
                    turned = jnp.broadcast_to(row, (T, T)).T
                    kv_ref[vtiles.index(t), d * VK : d * VK + n] = turned[:n]
            va_ref[0:16, _tile(t)] = _pack(_with_ones(y[32:64], False))
            va_ref[16:32, _tile(t)] = _pack(_with_ones(pltpu.roll(y[32:64], 4, 0), True))
        yield 128

        def queries(g, t, y):
            y = _pack(y * QSCALE)
            if t < TC and g < 2:
                stage_queries(g, t, y)
            else:
                qa_ref[g, :, _tile(t)] = y

        yield from each_group(wa_ref, 0, t0, ln, queries)

    def project_b(t0, ln, tails):
        block = _iota((T // 2, T), 1) // DH
        row_block = _iota((GD // 2, T), 0) // (DH // 2)
        lane_block = _iota((GD // 2, T), 1) // QW
        shifts = range(1 - G, G)

        def roll_heads(k):
            return {d: pltpu.roll(k, (d * DH) % T, 1) if d else k for d in shifts}

        def keys(g, t, y):
            k = _pack_transposed(_pad_rows(y))
            rolled = roll_heads(k)
            if t == 0:
                tails[g] = dict.fromkeys(shifts, jnp.zeros((LAG // 2, T), U32))
            elif g not in tails:
                tails[g] = roll_heads(tail_ref[g])
            if t + 1 == SPLIT:
                tail_ref[g] = k[QW // 2 :]
            win = {d: jnp.concatenate([tails[g][d], rolled[d]], axis=0) for d in shifts}
            tails[g] = {d: rolled[d][QW // 2 :] for d in shifts}
            for j in range(G):
                out = win[-j][0 : T // 2]
                for b in range(1, G):
                    r0 = b * QW // 2
                    out = jnp.where(block == b, win[b - j][r0 : r0 + T // 2], out)
                kb_ref[g * G + j, t * T // 2 : (t + 1) * T // 2, :] = out

        def queries(g, t, y):
            y = _pack(y * QSCALE)
            rolled = {
                d: pltpu.roll(y, (d * DH // 2) % (GD // 2), 0) if d else y for d in shifts
            }
            for j in range(G):
                parts = []
                for r in range(0, GD // 2, 8):
                    rows = slice(r, r + 8)
                    out = jnp.zeros((8, T), U32)
                    for b in range(r // (DH // 2), min((r + 7) // (DH // 2), G - 1) + 1):
                        here = (row_block[rows] == b) & (lane_block[rows] == b)
                        out = jnp.where(here, rolled[b - j][rows], out)
                    parts.append(out)
                q_ref[g * G + j, :, _tile(t)] = jnp.concatenate(parts, axis=0)

        def values(g, t, y):
            for j in range(G):
                h = g * G + j
                vb_ref[16 * h : 16 * (h + 1), _tile(t)] = _pack(
                    _with_ones(_window(y, j), j % 2)
                )

        yield from each_group(wb_ref, NG, t0, ln, keys, at_once=4)
        yield from each_group(wb_ref, 0, t0, ln, queries, at_once=2)
        yield from each_group(wb_ref, 2 * NG, t0, ln, values, at_once=2)

    def add_output(t0, o, wot_ref, dst_ref):
        def add(g, t, y):
            r = slice(g * GD, (g + 1) * GD)
            dst_ref[r, _tile(t)] = (x_ref[r, _tile(t)] + y).astype(dst_ref.dtype)

        yield from each_group(wot_ref, 0, t0, o, add)

    def a_queries(i, par):
        q = qa_ref[i % NG, :, chunk(i // NG)]
        for u in range(TC):
            stage_queries(par, u, q[:, _tile(u)])
            yield 1

    parts = [(j, u0) for u0 in range(0, TC, PART) for j in range(G)]

    def a_scores(par):
        s_ref, m_ref = bufs[par]
        for j, u0 in parts:
            tiles = range(u0, u0 + PART)
            q = _unpack(qh_refs[par][j, :, u0 * T : (u0 + PART) * T])
            mx = {}

            def record(u, keys, s):
                s_ref[j, keys, _tile(u)] = s
                for r in range(0, s.shape[0], 8):
                    mx[u] = jnp.maximum(mx[u], s[r : r + 8]) if u in mx else s[r : r + 8]

            def vector_scores():
                for n, t in enumerate(vtiles):
                    for u in tiles:
                        acc = None
                        for d in range(DH):
                            r = j * DH + d
                            keys = kv_ref[n, d * VK : (d + 1) * VK]
                            prod = keys * qf_refs[par][r : r + 1, _tile(u)]
                            acc = acc + prod if d else prod
                        record(u, slice((t + 1) * T - VK, (t + 1) * T), acc)
                        yield

            vector = vector_scores()
            total, done = NV * PART, 0
            for t in range(NT):
                k0, k1 = t * T, (t + 1) * T - (VK if t in vtiles else 0)
                s = _dot(_unpack(ka_ref[k0 // 2 : k1 // 2, 0:32]), q)
                yield PART / TC
                for r in range(k0, k1, 8):
                    for u in tiles:
                        record(u, slice(r, r + 8), s[r - k0 : r - k0 + 8, _tile(u - u0)])
                    while done < min(total, total * (r + 8) / (S - 72)):
                        next(vector)
                        done += 1
            for u in tiles:
                m_ref[j, 0:8, _tile(u)] = mx[u]

    def a_values(i, par):
        s_ref, m_ref = bufs[par]
        yield 0.01
        for j, u0 in parts:
            lanes = slice(u0 * T, (u0 + PART) * T)
            m = jnp.max(m_ref[j, 0:8, lanes], axis=0, keepdims=True)
            acc = None
            for t in range(NT):
                p = jnp.exp2(s_ref[j, _tile(t), lanes] - m).astype(BF16)
                a = _dot(_unpack(va_ref[16 * (j % 2) : 16 * (j % 2 + 1), _tile(t)]), p)
                acc = a if acc is None else acc + a
                if t == NT - 1:
                    col = (i // NG) * CH + u0 * T
                    col = col if isinstance(i, int) else pl.multiple_of(col, T)
                    o_ref[(i % NG) * G + j, :, pl.ds(col, PART * T)] = acc
                yield PART / TC

    b_parts = [(g, u, j) for g in range(NG) for u in range(TC) for j in range(G)]

    def b_scores(c):
        s_ref, m_ref = bufs[c % 2]
        causal = _iota((QW, T), 0) <= _iota((QW, T), 1) % QW
        for g, u, j in b_parts:
            t0 = c * CH + u * T
            h = g * G + j
            q = _unpack(q_ref[h, :, t0 : t0 + T])
            first, mx = MASKED, None
            for b0 in range(0, NB, 2):
                b1 = min(b0 + 2, NB)
                cost = 3 * (b1 - b0) / NB
                b0 = max(b0, (W - LAG - t0) // QW)
                if b0 < b1:
                    lo = (t0 - W + LAG + b0 * QW) // 2
                    keys = kb_ref[h, lo : lo + (b1 - b0) * QW // 2, 0:GD]
                    s = _dot(_unpack(keys), q)
                for band in range(b0, b1):
                    sb = s[(band - b0) * QW : (band - b0 + 1) * QW]
                    missing = (W - t0) // QW - band
                    if missing > 0:
                        sb = jnp.where(_iota(sb.shape, 1) >= missing * QW, sb, MASKED)
                    if band == 0:
                        first = sb
                        continue
                    r = g * W + band * QW
                    if band == NB - 1:
                        sb = jnp.where(causal, sb, first)
                        r = g * W
                    s_ref[j, r : r + QW, _tile(u)] = sb
                    s8 = jnp.max(sb.reshape(QW // 8, 8, T), axis=0)
                    mx = s8 if mx is None else jnp.maximum(mx, s8)
                if b1 == NB:
                    m_ref[j, 8 * g : 8 * g + 8, _tile(u)] = mx
                yield cost

    def b_values(c):
        s_ref, m_ref = bufs[c % 2]
        causal = _iota((QW, T), 0) <= _iota((QW, T), 1) % QW
        lane_block = _iota((QW, T), 1) // QW
        odd_block, high_block = lane_block % 2 == 1, lane_block // 2 == 1
        zero = jnp.zeros((QW, T), F32)
        yield 5

        def select(cond, a, b):
            if a is None and b is None:
                return None
            return jnp.where(cond, zero if a is None else a, zero if b is None else b)

        for g, u, j in b_parts:
            t0 = c * CH + u * T
            h = g * G + j
            m = jnp.max(m_ref[j, 8 * g : 8 * g + 8, _tile(u)], axis=0, keepdims=True)
            probs, halves, acc = {}, {}, None

            def prob(band):
                if band < max(0, (W - LAG - t0) // QW) or band >= NB:
                    return None
                if band not in probs:
                    r = g * W + (band % (NB - 1)) * QW
                    e = jnp.exp2(s_ref[j, r : r + QW, _tile(u)] - m)
                    if band in (0, NB - 1):
                        probs[0] = jnp.where(causal, 0.0, e)
                        probs[NB - 1] = jnp.where(causal, e, 0.0)
                    else:
                        probs[band] = e
                return probs[band]

            def half(band):
                if band not in halves:
                    halves[band] = select(odd_block, prob(band - 1), prob(band))
                return halves[band]

            for kt in range(W // T + 1):
                k0 = t0 - W + kt * T
                if k0 >= 0:
                    p = [
                        select(high_block, half(band - 2), half(band))
                        for band in range(kt * G, (kt + 1) * G)
                    ]
                    p = jnp.concatenate([zero if x is None else x for x in p], axis=0)
                    v = _unpack(vb_ref[16 * h : 16 * (h + 1), k0 : k0 + T])
                    a = _dot(v, p.astype(BF16))
                    acc = a if acc is None else acc + a
                if kt == W // T:
                    o_ref[h, :, t0 : t0 + T] = acc
                yield 1

    a_cost = G * NT
    b_cost = H * TC * (W // T + 1)

    def region(make_task):
        @pl.when(fence_ref[0] > 0)
        def _():
            for _ in make_task()[1]:
                pass

    def load_input(t0):
        ln = []
        for t in (t0, t0 + 1):
            x = xin_ref[:, _tile(t)].astype(F32)
            x_ref[:, _tile(t)] = x
            ln.append(_layernorm(x))
        return split(*ln)

    def first_project(t, ln):
        if t + 2 == FIRST:
            x_in[1].wait()
            for copy in w_in[3:]:
                copy.start()
        task = project_a(t, ln)
        yield next(task)
        if t == 0:
            yield from stage_weights(wq_ref, wa_ref)
        yield from task

    def stage_kv_weights():
        pad = jnp.zeros((4, D), F32)
        w = jnp.concatenate(
            [wkt_ref[...].astype(F32), pad, wvt_ref[...].astype(F32), pad], axis=0
        )
        wa_ref[D // 2 : D // 2 + 32, :] = _pack(
            jnp.concatenate([w[:, a:b] for a, b in depth], axis=1)
        )
        yield 1

    def stage_other_weights():
        yield from stage_weights(woa_ref, woat_ref)
        yield from stage_weights(wqkv_ref, wb_ref)
        yield from stage_weights(wob_ref, wobt_ref)

    def a_step(i, par, more=True):
        return _mixed(
            (a_cost, a_scores(1 - par)),
            (a_cost + 0.01, a_values(i, par)),
            *([(TC, a_queries(i + 2, par))] if more else []),
        )

    def a_steps(n, _):
        for _ in a_step(2 * n, 0)[1]:
            pass
        region(lambda: a_step(2 * n + 1, 1))

    def project_out(wot_ref, dst_ref, t0, t1):
        task = functools.partial(add_output, wot_ref=wot_ref, dst_ref=dst_ref)
        return D * (t1 - t0), tile_pairs(task, attended, t0, t1)

    def project_in_b(t0, t1):
        task = functools.partial(project_b, tails={})
        return 3 * D * (t1 - t0), tile_pairs(task, normed, t0, t1)

    def a_to_b():
        in_b = project_in_b(0, SPLIT)
        return _chain(
            _mixed(
                (a_cost, a_values(NC * NG - 1, 1)),
                _chain(
                    project_out(woat_ref, x_ref, 0, NT - TC),
                    _head(in_b, 3 * D * (SPLIT - 0.3)),
                ),
            ),
            project_out(woat_ref, x_ref, NT - TC, NT),
            in_b,
        )

    def b_step(c):
        return _mixed((b_cost, b_scores(c + 1)), (b_cost + 8, b_values(c)))

    def b_last(dst_ref, t0):
        return _mixed(
            (b_cost + 2, b_values(NC - 1)), project_out(wobt_ref, dst_ref, t0, NT - TC)
        )

    def b_to_a():
        return _chain(
            b_last(x_ref, 0),
            project_out(wobt_ref, x_ref, NT - TC, NT),
            (1, tile_pairs(project_a, normed, 0, NT)),
        )

    for copy in (x_in[0], *w_in[:3], x_in[1]):
        copy.start()
    fence_ref[0] = 1
    for copy in (x_in[0], *w_in[:3]):
        copy.wait()
    region(
        lambda: _chain(
            (1, stage_kv_weights()), (1, tile_pairs(first_project, load_input, 0, NT))
        )
    )
    for copy in w_in[3:]:
        copy.wait()

    for last in (False, True):
        region(
            lambda: _mixed(
                (a_cost, a_scores(0)), *([] if last else [(19, stage_other_weights())])
            )
        )
        lax.fori_loop(0, NC * NG // 2 - 1, a_steps, None)
        region(lambda: a_step(NC * NG - 2, 0, more=False))
        region(a_to_b)
        region(lambda: _chain((b_cost, b_scores(0)), project_in_b(SPLIT, NT)))
        for c in range(NC - 2):
            region(lambda: b_step(c))
        if last:
            region(lambda: _chain(b_step(NC - 2), project_out(wobt_ref, out_ref, 0, TC)))
            x_out[0].start()
            region(lambda: b_last(out_ref, TC))
            for copy in x_out[1:-1]:
                copy.start()
            region(lambda: project_out(wobt_ref, out_ref, NT - TC, NT))
            x_out[-1].start()
        else:
            region(lambda: b_step(NC - 2))
            region(b_to_a)
    for copy in x_out:
        copy.wait()


@jax.jit
def pallas_interleave_layers__grouped_kv_mqa__sliding_block__prompt_kernel(
    A_x: jax.Array,
    A_wq: jax.Array,
    A_wk: jax.Array,
    A_wv: jax.Array,
    A_wo: jax.Array,
    B_x: jax.Array,
    B_wqkv: jax.Array,
    B_wo: jax.Array,
):
    del B_x
    _, S, D = A_x.shape
    operands = (A_x[0].T, A_wq, A_wk.T, A_wv.T, A_wo, B_wqkv, B_wo)
    out_t = pl.pallas_call(
        _kernel,
        out_shape=jax.ShapeDtypeStruct((D, S), A_x.dtype),
        in_specs=[pl.BlockSpec(memory_space=pl.ANY)] * len(operands),
        out_specs=pl.BlockSpec(memory_space=pl.ANY),
        scratch_shapes=[
            *[pltpu.VMEM(a.shape, a.dtype) for a in operands],
            pltpu.VMEM((D, S), A_x.dtype),
            pltpu.VMEM((D, S), F32),
            pltpu.VMEM((D // 2 + 32, 5 * T), U32),
            pltpu.VMEM((3 * D // 2, 5 * T), U32),
            *[pltpu.VMEM((D // 2, 5 * T), U32)] * 2,
            pltpu.VMEM((S // 2, T), U32),
            pltpu.VMEM((NV, DH * VK, T), F32),
            pltpu.VMEM((32, S), U32),
            pltpu.VMEM((NG, GD // 2, S), U32),
            *[pltpu.VMEM((GD, CH), F32)] * 2,
            *[pltpu.VMEM((G, 16, CH), U32)] * 2,
            pltpu.VMEM((H, GD // 2, S), U32),
            pltpu.VMEM((H, S // 2, T), U32),
            pltpu.VMEM((NG, LAG // 2, T), U32),
            pltpu.VMEM((H * 16, S), U32),
            pltpu.VMEM((H, 32, S), F32),
            *[pltpu.VMEM((G, S, CH), F32)] * 2,
            *[pltpu.VMEM((G, 8 * NG, CH), F32)] * 2,
            pltpu.SMEM((1,), jnp.int32),
            pltpu.SemaphoreType.DMA((len(operands) + 1,)),
            pltpu.SemaphoreType.DMA((S // CH,)),
        ],
        compiler_params=pltpu.CompilerParams(
            vmem_limit_bytes=110 * 1024 * 1024,
            flags={"XLA_TPU_EVENLY_DISTRIBUTE_CRITICAL_NODES": True},
        ),
    )(*operands)
    return out_t.T[None]
```
